```python
import os as _os
_os.environ.setdefault('JAX_PLATFORMS', 'cpu')
import jax
import jax.numpy as jnp

def _softmax(x, axis=-1):
    return jax.nn.softmax(x, axis=axis)

def _gelu(x):
    return jax.nn.gelu(x, approximate=True)

def _silu(x):
    return jax.nn.silu(x)

def _sigmoid(x):
    return jax.nn.sigmoid(x)

def _layernorm(x, axis=-1, eps=1e-05):
    m = jnp.mean(x, axis=axis, keepdims=True)
    v = jnp.var(x, axis=axis, keepdims=True)
    return (x - m) / jnp.sqrt(v + eps)

def _scatter_add(tgt, idx, src, axis=0):
    return tgt.at[idx].add(src)

def _segment_sum(src, seg, n):
    return jax.ops.segment_sum(src, seg, n)

class _Rng:

    def __init__(self, key):
        self._k = key

    def _next(self):
        self._k, sub = jax.random.split(self._k)
        return sub

    def normal(self, shape):
        return jax.random.normal(self._next(), shape, dtype=jnp.bfloat16)

    def randint(self, lo, hi, shape):
        return jax.random.randint(self._next(), shape, lo, hi, dtype=jnp.int32)

    def uniform(self, shape, lo=0.0, hi=1.0):
        return jax.random.uniform(self._next(), shape, jnp.bfloat16, lo, hi)

    def permutation(self, n):
        return jax.random.permutation(self._next(), n)
kernel_name = 'gated_mix__mha_block__memory_aug_recurrent_mem_tr__prompt'

def setup_inputs():
    _rng = _Rng(jax.random.key(int.from_bytes(__import__("os").urandom(4), "little")))
    _w = lambda a: (lambda t: t.astype(jnp.bfloat16) if jnp.issubdtype(t.dtype, jnp.floating) else t)(jnp.asarray(a))

    def _A_setup():
        B, S, D, H = (1, 2048, 512, 32)
        return {'x': _w((lambda *s: _rng.normal(s) * 0.05)(B, S, D)), 'wqkv': _w((lambda *s: _rng.normal(s) * 0.8)(D, 3 * D)), 'wo': _w((lambda *s: _rng.normal(s) * 0.05)(D, D))}
    _A_in = _A_setup()

    def _B_setup():
        B, S, Dm = (1, 2048, 512)
        H, Dh = (32, 128)
        M, seg = (8, 32)
        seg = min(seg, S)
        S = S // seg * seg
        return {'x': _w((lambda *s: _rng.normal(s) * 0.05)(B, S, Dm)), 'mem0': _w((lambda *s: _rng.normal(s) * 0.8)(B, M, Dm)), 'Wq': _w((lambda *s: _rng.normal(s) * 1.6)(Dm, H, Dh) * Dm ** (-0.5)), 'Wk': _w((lambda *s: _rng.normal(s) * 1.6)(Dm, H, Dh) * Dm ** (-0.5)), 'Wv': _w((lambda *s: _rng.normal(s) * 0.8)(Dm, H, Dh) * Dm ** (-0.5)), 'Wo': _w((lambda *s: _rng.normal(s) * 0.8)(H, Dh, Dm) * (H * Dh) ** (-0.5)), 'seg_len': seg}
    _B_in = _B_setup()
    return {'A_x': _A_in['x'], 'A_wqkv': _A_in['wqkv'], 'A_wo': _A_in['wo'], 'B_x': _B_in['x'], 'B_mem0': _B_in['mem0'], 'B_Wq': _B_in['Wq'], 'B_Wk': _B_in['Wk'], 'B_Wv': _B_in['Wv'], 'B_Wo': _B_in['Wo'], 'B_seg_len': _B_in['seg_len'], 'gate_w': _w((lambda *s: _rng.normal(s) * 0.05)(512) * 16.0)}

def reference(A_x, A_wqkv, A_wo, B_x, B_mem0, B_Wq, B_Wk, B_Wv, B_Wo, B_seg_len, gate_w):

    def _A_ref(x, wqkv, wo):
        B, S, D = x.shape
        H = 32
        Dh = D // H
        qkv = (lambda x, *d: x.transpose(*d))((x @ wqkv).reshape(B, S, 3, H, Dh), 2, 0, 3, 1, 4)
        q, k, v = (qkv[0], qkv[1], qkv[2])
        scores = jnp.einsum('bhqd,bhkd->bhqk', q, k) * Dh ** (-0.5)
        p = _softmax(scores, axis=-1)
        o = jnp.einsum('bhqk,bhkd->bhqd', p, v)
        return (lambda x, *d: x.transpose(*d))(o, 0, 2, 1, 3).reshape(B, S, D) @ wo

    def _B_ref(x, mem0, Wq, Wk, Wv, Wo, seg_len):
        B, S, Dm = x.shape
        H, Dh = (Wq.shape[1], Wq.shape[2])
        M = mem0.shape[1]
        scale = Dh ** (-0.5)
        n_seg = S // seg_len
        L = M + seg_len
        idx = jnp.arange(L)
        mask = (idx[:, None] < M) | (idx[:, None] >= idx[None, :])
        mem = mem0
        outs = []
        for s in range(n_seg):
            xs = x[:, s * seg_len:(s + 1) * seg_len, :].copy()
            h = jnp.concatenate([mem, xs], axis=1)
            q = jnp.einsum('btd,dhe->bhte', h, Wq)
            k = jnp.einsum('btd,dhe->bhte', h, Wk)
            v = jnp.einsum('btd,dhe->bhte', h, Wv)
            scores = jnp.einsum('bhqe,bhke->bhqk', q, k) * scale
            scores = jnp.where(mask[None, None], scores, -1000000000.0)
            p = _softmax(scores, axis=-1)
            o = jnp.einsum('bhqk,bhke->bhqe', p, v)
            o = jnp.einsum('bhte,hed->btd', o, Wo)
            mem = o[:, :M, :].copy()
            outs.append(o[:, M:, :])
        return jnp.concatenate(outs, axis=1)
    x = A_x
    g = _sigmoid((x * gate_w).sum(-1, keepdims=True))
    a = _A_ref(x, A_wqkv, A_wo)
    b = _B_ref(x, B_mem0, B_Wq, B_Wk, B_Wv, B_Wo, B_seg_len)
    return g * a + (1 - g) * b
```

```python
import functools
import math

import jax
import jax.numpy as jnp
from jax import lax
from jax.experimental import pallas as pl
from jax.experimental.pallas import tpu as pltpu

F32 = jnp.float32
BF16 = jnp.bfloat16
LOG2E = math.log2(math.e)

SAFE_LOG2 = 64.0


def _dot(a, b):
    return lax.dot_general(a, b, (((1,), (0,)), ((), ())), preferred_element_type=F32)


def _dot_nt(a, b):
    return lax.dot_general(a, b, (((1,), (1,)), ((), ())), preferred_element_type=F32)


def _dot_tn(a, b):
    return lax.dot_general(a, b, (((0,), (0,)), ((), ())), preferred_element_type=F32)


def _make_kernel(S, D, HA, HB, EB, M, SEG):
    DA = D // HA
    HPG = 128 // DA
    NG = D // 128
    BQ = 512
    BK = 128
    NQ = S // BQ
    NBLK = HA * NQ
    NSEG = S // SEG
    L = M + SEG
    cA = (DA ** -0.5) * LOG2E
    cB = (EB ** -0.5) * LOG2E

    def kernel(x_hbm, wqkv_hbm, wo_hbm, mem0_ref, wq_hbm, wk_hbm, wv_hbm, woB_hbm, gw_ref,
               out_ref,
               x_v, wqkv_v, wo_v, st_v, woB_v, wB_v,
               k_v, qt_v, vt_v, pa_v, pb_v, ot_v, b_v, sems):
        cp_x = pltpu.make_async_copy(x_hbm, x_v, sems.at[0])
        cp_wqkv = pltpu.make_async_copy(wqkv_hbm, wqkv_v, sems.at[1])
        cp_wo = pltpu.make_async_copy(wo_hbm, wo_v, sems.at[2])
        cp_w = [
            pltpu.make_async_copy(w.bitcast(jnp.uint32), st_v.at[i], sems.at[3 + i])
            for i, w in enumerate((wq_hbm, wk_hbm, wv_hbm))
        ]
        cp_woB = pltpu.make_async_copy(woB_hbm, woB_v, sems.at[6])
        cp_x.start()
        cp_wqkv.start()
        for c in cp_w:
            c.start()
        cp_woB.start()
        cp_wo.start()
        cp_x.wait()
        cp_wqkv.wait()

        esel = (lax.broadcasted_iota(jnp.int32, (HA, D), 1) // DA
                == lax.broadcasted_iota(jnp.int32, (HA, D), 0)).astype(BF16)
        kn2 = jnp.zeros((HA, S), F32)
        for g in range(NG):
            kg = _dot(x_v[...], wqkv_v[:, D + g * 128:D + (g + 1) * 128]).astype(BF16)
            k_v[g] = kg
            kf = kg.astype(F32)
            kn2 = kn2 + _dot_nt(esel[:, g * 128:(g + 1) * 128], (kf * kf).astype(BF16))
        qn2 = jnp.zeros((HA, S), F32)
        for g in range(NG):
            wq_g = wqkv_v[:, g * 128:(g + 1) * 128]
            qg = (lax.dot_general(wq_g, x_v[...], (((0,), (1,)), ((), ())),
                                  preferred_element_type=F32) * cA).astype(BF16)
            qt_v[g * 128:(g + 1) * 128, :] = qg
            qf = qg.astype(F32)
            qn2 = qn2 + _dot(esel[:, g * 128:(g + 1) * 128], (qf * qf).astype(BF16))
            wv_g = wqkv_v[:, 2 * D + g * 128:2 * D + (g + 1) * 128]
            vg = lax.dot_general(wv_g, x_v[...], (((0,), (1,)), ((), ())),
                                 preferred_element_type=F32).astype(BF16)
            for j in range(HPG):
                vt_v[g * HPG + j] = vg[j * DA:(j + 1) * DA, :]
        bound2 = jnp.max(qn2) * jnp.max(kn2) * 1.02
        safe = bound2 <= SAFE_LOG2 * SAFE_LOG2

        def masked_q(h, qb):
            g = h // HPG
            j = h % HPG
            q0 = pl.multiple_of(qb * BQ, BQ)
            g0 = pl.multiple_of(g * 128, 128)
            qt = qt_v[pl.ds(g0, 128), pl.ds(q0, BQ)]
            row = lax.broadcasted_iota(jnp.int32, (128, BQ), 0)
            return g, jnp.where((row >= j * DA) & (row < (j + 1) * DA), qt, jnp.zeros_like(qt))

        def block(it, p_cur, p_prev, l_prev, do_qk, do_pv):
            if do_qk:
                h, qb = it // NQ, it % NQ
                g, qtm = masked_q(h, qb)
                l = jnp.zeros((8, BQ), F32)
            if do_pv:
                hp, qbp = (it - 1) // NQ, (it - 1) % NQ
                acc = jnp.zeros((DA, BQ), F32)
            for kc in range(S // BK):
                ks = pl.ds(kc * BK, BK)
                if do_qk:
                    s = _dot(k_v[g, ks, :], qtm)
                    p = jnp.exp2(s)
                    l = l + p.reshape(BK // 8, 8, BQ).sum(axis=0)
                    p_cur[ks, :] = p.astype(BF16)
                if do_pv:
                    acc = acc + _dot(vt_v[hp, :, ks], p_prev[ks, :])
            if do_pv:
                lsum = jnp.sum(l_prev, axis=0, keepdims=True)
                o = acc * (1.0 / lsum)
                ot_v[pl.ds(pl.multiple_of(hp * DA, DA), DA), pl.ds(pl.multiple_of(qbp * BQ, BQ), BQ)] = o.astype(BF16)
            return l if do_qk else None

        @pl.when(safe)
        def _fast():
            l0 = block(0, pa_v, None, None, True, False)

            def body(i2, l):
                l = block(2 * i2 + 1, pb_v, pa_v, l, True, True)
                l = block(2 * i2 + 2, pa_v, pb_v, l, True, True)
                return l

            l = lax.fori_loop(0, NBLK // 2 - 1, body, l0)
            l = block(NBLK - 1, pb_v, pa_v, l, True, True)
            block(NBLK, None, pb_v, l, False, True)

        @pl.when(jnp.logical_not(safe))
        def _true_max():
            def body(it, c):
                h, qb = it // NQ, it % NQ
                g, qtm = masked_q(h, qb)

                def max_body(kc, m):
                    ks = pl.ds(pl.multiple_of(kc * 256, 256), 256)
                    s = _dot(k_v[g, ks, :], qtm)
                    return jnp.maximum(m, jnp.max(s, axis=0, keepdims=True))

                m = lax.fori_loop(0, S // 256, max_body, jnp.full((1, BQ), -jnp.inf, F32))

                def pv_body(kc, carry):
                    l, acc = carry
                    ks = pl.ds(pl.multiple_of(kc * 256, 256), 256)
                    s = _dot(k_v[g, ks, :], qtm)
                    p = jnp.exp2(s - m)
                    l = l + jnp.sum(p, axis=0, keepdims=True)
                    acc = acc + _dot(vt_v[h, :, ks], p.astype(BF16))
                    return l, acc

                l, acc = lax.fori_loop(0, S // 256, pv_body,
                                       (jnp.zeros((1, BQ), F32), jnp.zeros((DA, BQ), F32)))
                o = acc * (1.0 / l)
                ot_v[pl.ds(pl.multiple_of(h * DA, DA), DA), pl.ds(pl.multiple_of(qb * BQ, BQ), BQ)] = o.astype(BF16)
                return c

            lax.fori_loop(0, NBLK, body, 0)

        for c in cp_w:
            c.wait()
        cp_woB.wait()
        NP = HB // 2

        def relayout_body(i, c):
            for w in range(3):
                for dc in range(D // 128):
                    u = st_v[w, pl.ds(dc * 128 * NP + i, 128, stride=NP), :]
                    lo = pltpu.bitcast(u << 16, F32).astype(BF16)
                    hi = pltpu.bitcast(u & jnp.uint32(0xFFFF0000), F32).astype(BF16)
                    wB_v[w * HB + 2 * i, dc * 128:(dc + 1) * 128, :] = lo
                    wB_v[w * HB + 2 * i + 1, dc * 128:(dc + 1) * 128, :] = hi
            return c

        lax.fori_loop(0, NP, relayout_body, 0)

        ri = lax.broadcasted_iota(jnp.int32, (L, L), 0)
        ci = lax.broadcasted_iota(jnp.int32, (L, L), 1)
        mask = (ri < M) | (ri >= ci)

        def step(s, mem):
            r0 = pl.multiple_of(s * SEG, SEG)
            xs = x_v[pl.ds(r0, SEG), :].astype(F32)
            h = jnp.concatenate([mem, xs], axis=0)
            out = jnp.zeros((L, D), F32)
            for hd in range(HB):
                q = _dot(h, wB_v[hd])
                k = _dot(h, wB_v[HB + hd]).astype(BF16)
                v = _dot(h, wB_v[2 * HB + hd]).astype(BF16)
                sc = _dot_nt(q, k) * cB
                sc = jnp.where(mask, sc, -1e9)
                m = jnp.max(sc, axis=1, keepdims=True)
                p = jnp.exp2(sc - m)
                l = jnp.sum(p, axis=1, keepdims=True)
                o = _dot(p, v) * (1.0 / l)
                out = out + _dot(o, woB_v[hd * EB:(hd + 1) * EB, :])
            b_v[pl.ds(r0, SEG), :] = out[M:, :]
            return out[:M, :].astype(BF16).astype(F32)

        lax.fori_loop(0, NSEG, step, mem0_ref[...].astype(F32))

        cp_wo.wait()
        gw = gw_ref[...].astype(F32)
        RB = 256

        def fin(i, c):
            r0 = pl.multiple_of(i * RB, RB)
            xs = x_v[pl.ds(r0, RB), :].astype(F32)
            gate = jax.nn.sigmoid(jnp.sum(xs * gw, axis=1, keepdims=True))
            a = _dot_tn(ot_v[:, pl.ds(r0, RB)], wo_v[...])
            b = b_v[pl.ds(r0, RB), :]
            out_ref[pl.ds(r0, RB), :] = (gate * a + (1.0 - gate) * b).astype(out_ref.dtype)
            return c

        lax.fori_loop(0, S // RB, fin, 0)

    return kernel


@functools.partial(jax.jit, static_argnames=("B_seg_len",))
def pallas_gated_mix__mha_block__memory_aug_recurrent_mem_tr__prompt_kernel(
    A_x, A_wqkv, A_wo, B_x, B_mem0, B_Wq, B_Wk, B_Wv, B_Wo, B_seg_len, gate_w,
):
    del B_x
    Bsz, S, D = A_x.shape
    assert Bsz == 1
    HA = 32
    _, HB, EB = B_Wq.shape
    M = B_mem0.shape[1]
    SEG = int(B_seg_len)

    x = A_x.reshape(S, D)
    kernel = _make_kernel(S, D, HA, HB, EB, M, SEG)
    any_spec = pl.BlockSpec(memory_space=pl.ANY)
    vmem_spec = pl.BlockSpec(memory_space=pltpu.VMEM)
    out = pl.pallas_call(
        kernel,
        out_shape=jax.ShapeDtypeStruct((S, D), A_x.dtype),
        in_specs=[any_spec, any_spec, any_spec, vmem_spec, any_spec, any_spec, any_spec, any_spec, vmem_spec],
        out_specs=vmem_spec,
        scratch_shapes=[
            pltpu.VMEM((S, D), BF16),
            pltpu.VMEM((D, 3 * D), BF16),
            pltpu.VMEM((D, D), BF16),
            pltpu.VMEM((3, D * HB // 2, EB), jnp.uint32),
            pltpu.VMEM((HB * EB, D), BF16),
            pltpu.VMEM((3 * HB, D, EB), BF16),
            pltpu.VMEM((D // 128, S, 128), BF16),
            pltpu.VMEM((D, S), BF16),
            pltpu.VMEM((HA, D // HA, S), BF16),
            pltpu.VMEM((S, 512), BF16),
            pltpu.VMEM((S, 512), BF16),
            pltpu.VMEM((D, S), BF16),
            pltpu.VMEM((S, D), F32),
            pltpu.SemaphoreType.DMA((7,)),
        ],
        compiler_params=pltpu.CompilerParams(vmem_limit_bytes=100 * 1024 * 1024),
    )(
        x, A_wqkv, A_wo, B_mem0.reshape(M, D),
        B_Wq.reshape(D * HB, EB), B_Wk.reshape(D * HB, EB), B_Wv.reshape(D * HB, EB),
        B_Wo.reshape(HB * EB, D), gate_w.reshape(1, D),
    )
    return out.reshape(Bsz, S, D)
```

```python
import functools
import math

import jax
import jax.numpy as jnp
from jax import lax
from jax.experimental import pallas as pl
from jax.experimental.pallas import tpu as pltpu

F32 = jnp.float32
BF16 = jnp.bfloat16
LOG2E = math.log2(math.e)

SAFE_LOG2 = 64.0


def _dot(a, b):
    return lax.dot_general(a, b, (((1,), (0,)), ((), ())), preferred_element_type=F32)


def _dot_nt(a, b):
    return lax.dot_general(a, b, (((1,), (1,)), ((), ())), preferred_element_type=F32)


def _dot_tn(a, b):
    return lax.dot_general(a, b, (((0,), (0,)), ((), ())), preferred_element_type=F32)


def _make_kernel(S, D, HA, HB, EB, M, SEG):
    DA = D // HA
    HPG = 128 // DA
    NG = D // 128
    BQ = 512
    BK = 128
    NQ = S // BQ
    NBLK = HA * NQ
    NSEG = S // SEG
    L = M + SEG
    cA = (DA ** -0.5) * LOG2E
    cB = (EB ** -0.5) * LOG2E

    def kernel(x_hbm, wqkv_hbm, wo_hbm, mem0_ref, wq_hbm, wk_hbm, wv_hbm, woB_hbm, gw_ref,
               out_ref,
               x_v, wqkv_v, wo_v, st_v, woB_v, wB_v,
               k_v, qt_v, vt_v, pa_v, pb_v, ot_v, b_v, q_s, k_s, v_s, o_s, sems):
        cp_x = pltpu.make_async_copy(x_hbm, x_v, sems.at[0])
        cp_wqkv = pltpu.make_async_copy(wqkv_hbm, wqkv_v, sems.at[1])
        cp_wo = pltpu.make_async_copy(wo_hbm, wo_v, sems.at[2])
        cp_w = [
            pltpu.make_async_copy(w.bitcast(jnp.uint32), st_v.at[i], sems.at[3 + i])
            for i, w in enumerate((wq_hbm, wk_hbm, wv_hbm))
        ]
        cp_woB = pltpu.make_async_copy(woB_hbm, woB_v, sems.at[6])
        cp_x.start()
        cp_wqkv.start()
        for c in cp_w:
            c.start()
        cp_woB.start()
        cp_wo.start()
        cp_x.wait()
        cp_wqkv.wait()

        esel = (lax.broadcasted_iota(jnp.int32, (HA, D), 1) // DA
                == lax.broadcasted_iota(jnp.int32, (HA, D), 0)).astype(BF16)
        kn2 = jnp.zeros((HA, S), F32)
        for g in range(NG):
            kg = _dot(x_v[...], wqkv_v[:, D + g * 128:D + (g + 1) * 128]).astype(BF16)
            k_v[g] = kg
            kf = kg.astype(F32)
            kn2 = kn2 + _dot_nt(esel[:, g * 128:(g + 1) * 128], (kf * kf).astype(BF16))
        qn2 = jnp.zeros((HA, S), F32)
        for g in range(NG):
            wq_g = wqkv_v[:, g * 128:(g + 1) * 128]
            qg = (lax.dot_general(wq_g, x_v[...], (((0,), (1,)), ((), ())),
                                  preferred_element_type=F32) * cA).astype(BF16)
            qt_v[g * 128:(g + 1) * 128, :] = qg
            qf = qg.astype(F32)
            qn2 = qn2 + _dot(esel[:, g * 128:(g + 1) * 128], (qf * qf).astype(BF16))
            wv_g = wqkv_v[:, 2 * D + g * 128:2 * D + (g + 1) * 128]
            vg = lax.dot_general(wv_g, x_v[...], (((0,), (1,)), ((), ())),
                                 preferred_element_type=F32).astype(BF16)
            for j in range(HPG):
                vt_v[g * HPG + j] = vg[j * DA:(j + 1) * DA, :]
        bound2 = jnp.max(qn2) * jnp.max(kn2) * 1.02
        safe = bound2 <= SAFE_LOG2 * SAFE_LOG2

        def masked_q(h, qb):
            g = h // HPG
            j = h % HPG
            q0 = pl.multiple_of(qb * BQ, BQ)
            g0 = pl.multiple_of(g * 128, 128)
            qt = qt_v[pl.ds(g0, 128), pl.ds(q0, BQ)]
            row = lax.broadcasted_iota(jnp.int32, (128, BQ), 0)
            return g, jnp.where((row >= j * DA) & (row < (j + 1) * DA), qt, jnp.zeros_like(qt))

        def block(it, p_cur, p_prev, l_prev, do_qk, do_pv):
            if do_qk:
                h, qb = it // NQ, it % NQ
                g, qtm = masked_q(h, qb)
                l = jnp.zeros((8, BQ), F32)
            if do_pv:
                hp, qbp = (it - 1) // NQ, (it - 1) % NQ
                acc = jnp.zeros((DA, BQ), F32)
            for kc in range(S // BK):
                ks = pl.ds(kc * BK, BK)
                if do_qk:
                    s = _dot(k_v[g, ks, :], qtm)
                    p = jnp.exp2(s)
                    l = l + p.reshape(BK // 8, 8, BQ).sum(axis=0)
                    p_cur[ks, :] = p.astype(BF16)
                if do_pv:
                    acc = acc + _dot(vt_v[hp, :, ks], p_prev[ks, :])
            if do_pv:
                lsum = jnp.sum(l_prev, axis=0, keepdims=True)
                o = acc * (1.0 / lsum)
                ot_v[pl.ds(pl.multiple_of(hp * DA, DA), DA), pl.ds(pl.multiple_of(qbp * BQ, BQ), BQ)] = o.astype(BF16)
            return l if do_qk else None

        @pl.when(safe)
        def _fast():
            l0 = block(0, pa_v, None, None, True, False)

            def body(i2, l):
                l = block(2 * i2 + 1, pb_v, pa_v, l, True, True)
                l = block(2 * i2 + 2, pa_v, pb_v, l, True, True)
                return l

            l = lax.fori_loop(0, NBLK // 2 - 1, body, l0)
            l = block(NBLK - 1, pb_v, pa_v, l, True, True)
            block(NBLK, None, pb_v, l, False, True)

        @pl.when(jnp.logical_not(safe))
        def _true_max():
            def body(it, c):
                h, qb = it // NQ, it % NQ
                g, qtm = masked_q(h, qb)

                def max_body(kc, m):
                    ks = pl.ds(pl.multiple_of(kc * 256, 256), 256)
                    s = _dot(k_v[g, ks, :], qtm)
                    return jnp.maximum(m, jnp.max(s, axis=0, keepdims=True))

                m = lax.fori_loop(0, S // 256, max_body, jnp.full((1, BQ), -jnp.inf, F32))

                def pv_body(kc, carry):
                    l, acc = carry
                    ks = pl.ds(pl.multiple_of(kc * 256, 256), 256)
                    s = _dot(k_v[g, ks, :], qtm)
                    p = jnp.exp2(s - m)
                    l = l + jnp.sum(p, axis=0, keepdims=True)
                    acc = acc + _dot(vt_v[h, :, ks], p.astype(BF16))
                    return l, acc

                l, acc = lax.fori_loop(0, S // 256, pv_body,
                                       (jnp.zeros((1, BQ), F32), jnp.zeros((DA, BQ), F32)))
                o = acc * (1.0 / l)
                ot_v[pl.ds(pl.multiple_of(h * DA, DA), DA), pl.ds(pl.multiple_of(qb * BQ, BQ), BQ)] = o.astype(BF16)
                return c

            lax.fori_loop(0, NBLK, body, 0)

        for c in cp_w:
            c.wait()
        cp_woB.wait()
        NP = HB // 2

        def relayout_body(i, c):
            for w in range(3):
                for dc in range(D // 128):
                    u = st_v[w, pl.ds(dc * 128 * NP + i, 128, stride=NP), :]
                    lo = pltpu.bitcast(u << 16, F32).astype(BF16)
                    hi = pltpu.bitcast(u & jnp.uint32(0xFFFF0000), F32).astype(BF16)
                    wB_v[w * HB + 2 * i, dc * 128:(dc + 1) * 128, :] = lo
                    wB_v[w * HB + 2 * i + 1, dc * 128:(dc + 1) * 128, :] = hi
            return c

        lax.fori_loop(0, NP, relayout_body, 0)

        ri = lax.broadcasted_iota(jnp.int32, (L, L), 0)
        ci = lax.broadcasted_iota(jnp.int32, (L, L), 1)
        mask = (ri < M) | (ri >= ci)

        def step(s, mem):
            r0 = pl.multiple_of(s * SEG, SEG)
            xs = x_v[pl.ds(r0, SEG), :].astype(F32)
            h = jnp.concatenate([mem, xs], axis=0)
            for hd in range(HB):
                q_s[hd] = _dot(h, wB_v[hd])
                k_s[hd] = _dot(h, wB_v[HB + hd]).astype(BF16)
                v_s[hd] = _dot(h, wB_v[2 * HB + hd]).astype(BF16)
            pls = []
            for hd in range(HB):
                sc = _dot_nt(q_s[hd], k_s[hd]) * cB
                sc = jnp.where(mask, sc, -1e9)
                m = jnp.max(sc, axis=1, keepdims=True)
                p = jnp.exp2(sc - m)
                l = jnp.sum(p, axis=1, keepdims=True)
                pls.append((p, l))
            for hd in range(HB):
                p, l = pls[hd]
                o_s[hd] = _dot(p, v_s[hd]) * pl.reciprocal(l, approx=True)
            out = jnp.zeros((L, D), F32)
            for hd in range(HB):
                out = out + _dot(o_s[hd], woB_v[hd * EB:(hd + 1) * EB, :])
            b_v[pl.ds(r0, SEG), :] = out[M:, :]
            return out[:M, :].astype(BF16).astype(F32)

        lax.fori_loop(0, NSEG, step, mem0_ref[...].astype(F32))

        cp_wo.wait()
        gw = gw_ref[...].astype(F32)
        RB = 256

        def fin(i, c):
            r0 = pl.multiple_of(i * RB, RB)
            xs = x_v[pl.ds(r0, RB), :].astype(F32)
            gate = jax.nn.sigmoid(jnp.sum(xs * gw, axis=1, keepdims=True))
            a = _dot_tn(ot_v[:, pl.ds(r0, RB)], wo_v[...])
            b = b_v[pl.ds(r0, RB), :]
            out_ref[pl.ds(r0, RB), :] = (gate * a + (1.0 - gate) * b).astype(out_ref.dtype)
            return c

        lax.fori_loop(0, S // RB, fin, 0)

    return kernel


@functools.partial(jax.jit, static_argnames=("B_seg_len",))
def pallas_gated_mix__mha_block__memory_aug_recurrent_mem_tr__prompt_kernel(
    A_x, A_wqkv, A_wo, B_x, B_mem0, B_Wq, B_Wk, B_Wv, B_Wo, B_seg_len, gate_w,
):
    del B_x
    Bsz, S, D = A_x.shape
    assert Bsz == 1
    HA = 32
    _, HB, EB = B_Wq.shape
    M = B_mem0.shape[1]
    SEG = int(B_seg_len)

    x = A_x.reshape(S, D)
    kernel = _make_kernel(S, D, HA, HB, EB, M, SEG)
    any_spec = pl.BlockSpec(memory_space=pl.ANY)
    vmem_spec = pl.BlockSpec(memory_space=pltpu.VMEM)
    out = pl.pallas_call(
        kernel,
        out_shape=jax.ShapeDtypeStruct((S, D), A_x.dtype),
        in_specs=[any_spec, any_spec, any_spec, vmem_spec, any_spec, any_spec, any_spec, any_spec, vmem_spec],
        out_specs=vmem_spec,
        scratch_shapes=[
            pltpu.VMEM((S, D), BF16),
            pltpu.VMEM((D, 3 * D), BF16),
            pltpu.VMEM((D, D), BF16),
            pltpu.VMEM((3, D * HB // 2, EB), jnp.uint32),
            pltpu.VMEM((HB * EB, D), BF16),
            pltpu.VMEM((3 * HB, D, EB), BF16),
            pltpu.VMEM((D // 128, S, 128), BF16),
            pltpu.VMEM((D, S), BF16),
            pltpu.VMEM((HA, D // HA, S), BF16),
            pltpu.VMEM((S, 512), BF16),
            pltpu.VMEM((S, 512), BF16),
            pltpu.VMEM((D, S), BF16),
            pltpu.VMEM((S, D), F32),
            pltpu.VMEM((HB, M + SEG, EB), F32),
            pltpu.VMEM((HB, M + SEG, EB), BF16),
            pltpu.VMEM((HB, M + SEG, EB), BF16),
            pltpu.VMEM((HB, M + SEG, EB), F32),
            pltpu.SemaphoreType.DMA((7,)),
        ],
        compiler_params=pltpu.CompilerParams(vmem_limit_bytes=100 * 1024 * 1024),
    )(
        x, A_wqkv, A_wo, B_mem0.reshape(M, D),
        B_Wq.reshape(D * HB, EB), B_Wk.reshape(D * HB, EB), B_Wv.reshape(D * HB, EB),
        B_Wo.reshape(HB * EB, D), gate_w.reshape(1, D),
    )
    return out.reshape(Bsz, S, D)
```

```python
import functools
import math

import jax
import jax.numpy as jnp
from jax import lax
from jax.experimental import pallas as pl
from jax.experimental.pallas import tpu as pltpu

F32 = jnp.float32
BF16 = jnp.bfloat16
LOG2E = math.log2(math.e)

L_MIN = 2.0 ** -32
L_MAX = 2.0 ** 64
O_MAX = 3.0e38
UNROLL = 2


def _dot(a, b):
    return lax.dot_general(a, b, (((1,), (0,)), ((), ())), preferred_element_type=F32)


def _dot_nt(a, b):
    return lax.dot_general(a, b, (((1,), (1,)), ((), ())), preferred_element_type=F32)


def _dot_tn(a, b):
    return lax.dot_general(a, b, (((0,), (0,)), ((), ())), preferred_element_type=F32)


def _dot_tt(a, b):
    return lax.dot_general(a, b, (((0,), (1,)), ((), ())), preferred_element_type=F32)


def _make_kernel(S, D, HA, HB, EB, M, SEG, scope):
    DA = D // HA
    HPG = 128 // DA
    NG = D // 128
    BQ = 512
    BK = 128
    NC = S // BK
    NQ = S // BQ
    NBLK = HA * NQ
    NSEG = S // SEG
    L = M + SEG
    NP = HB // 2
    XC = 512
    NXC = S // XC
    PITCH = 24
    NPRE = 3
    NFUSE = NSEG - NXC
    assert 2 + 2 * NPRE + 2 * NFUSE == NBLK
    cA = (DA ** -0.5) * LOG2E
    cB = (EB ** -0.5) * LOG2E

    def kernel(x_hbm, wqkv_hbm, wo_hbm, mem0_hbm, wq_hbm, wk_hbm, wv_hbm, woB_hbm, gw_hbm,
               out_hbm,
               mem0_v, gw_v, x_v, wqkv_v, wo_v, st_v, woB_v, wB_v, wqT_v, wvT_v,
               k_v, qt_v, vt_v, pa_v, pb_v, ot_v, b_v, o_v, mem_v, l_v, bad_v, alast_v, glast_v,
               q_s, k_s, v_s, o_s, sems, osems):
        cp_wa = [pltpu.make_async_copy(wqkv_hbm.at[:, pl.ds(i * D, D)], wqkv_v.at[i], sems.at[i]) for i in range(3)]

        def x_copy(c):
            cs = pl.ds(pl.multiple_of(c * XC, XC), XC)
            return pltpu.make_async_copy(x_hbm.at[cs], x_v.at[cs], sems.at[3 + c])

        cp_x = [x_copy(c) for c in range(NXC)]
        cp_w = [
            pltpu.make_async_copy(w.bitcast(jnp.uint32), st_v.at[i, :, pl.ds(0, NP), :], sems.at[3 + NXC + i])
            for i, w in enumerate((wq_hbm, wk_hbm, wv_hbm))
        ]
        cp_woB = pltpu.make_async_copy(woB_hbm, woB_v, sems.at[6 + NXC])
        cp_wo = pltpu.make_async_copy(wo_hbm, wo_v, sems.at[7 + NXC])
        cp_mem = pltpu.make_async_copy(mem0_hbm, mem0_v, sems.at[8 + NXC])
        cp_gw = pltpu.make_async_copy(gw_hbm, gw_v, sems.at[9 + NXC])
        for cp in [cp_wa[1]] + cp_x + [cp_wa[0], cp_wa[2], cp_mem, cp_gw] + cp_w + [cp_woB, cp_wo]:
            cp.start()

        with scope("P1_Aproj"):
            with scope("P1w"):
                cp_wa[1].wait()

            def k_body(c, carry):
                cs = pl.ds(pl.multiple_of(c * XC, XC), XC)
                x_copy(c).wait()
                xc = x_v[cs, :]
                for g in range(NG):
                    k_v[g, cs, :] = _dot(xc, wqkv_v[1, :, g * 128:(g + 1) * 128]).astype(BF16)
                return carry

            lax.fori_loop(0, NXC, k_body, 0)
            cp_wa[0].wait()
            cp_wa[2].wait()

            def qv_body(c, carry):
                cs = pl.ds(pl.multiple_of(c * XC, XC), XC)
                xc = x_v[cs, :]
                qt_v[:, cs] = (_dot_tt(wqkv_v[0], xc) * cA).astype(BF16)
                vc = _dot_tt(wqkv_v[2], xc).astype(BF16)
                for hh in range(HA):
                    vt_v[hh, :, cs] = vc[hh * DA:(hh + 1) * DA, :]
                return carry

            lax.fori_loop(0, NXC, qv_body, 0)
            bad_v[...] = jnp.zeros_like(bad_v)

        def masked_q(h, qb):
            g = h // HPG
            j = h % HPG
            q0 = pl.multiple_of(qb * BQ, BQ)
            g0 = pl.multiple_of(g * 128, 128)
            qt = qt_v[pl.ds(g0, 128), pl.ds(q0, BQ)]
            row = lax.broadcasted_iota(jnp.int32, (128, BQ), 0)
            return g, jnp.where((row >= j * DA) & (row < (j + 1) * DA), qt, jnp.zeros_like(qt))

        def store_o(h, qb, o):
            ot_v[pl.ds(pl.multiple_of(h * DA, DA), DA), pl.ds(pl.multiple_of(qb * BQ, BQ), BQ)] = o.astype(BF16)

        class Slot:
            def __init__(self, t, p_cur, p_prev, l_prev):
                self.p_cur, self.p_prev, self.l_prev = p_cur, p_prev, l_prev
                self.kc = 0
                if p_cur is not None:
                    self.g, self.qtm = masked_q(t // NQ, t % NQ)
                    self.l = jnp.zeros((8, BQ), F32)
                if p_prev is not None:
                    self.hp, self.qbp = (t - 1) // NQ, (t - 1) % NQ
                    self.acc = jnp.zeros((DA, BQ), F32)

            def chunk(self):
                ks = pl.ds(self.kc * BK, BK)
                if self.p_cur is not None:
                    p = jnp.exp2(_dot(k_v[self.g, ks, :], self.qtm))
                    self.l = self.l + p.reshape(BK // 8, 8, BQ).sum(axis=0)
                    self.p_cur[ks, :] = p.astype(BF16)
                if self.p_prev is not None:
                    self.acc = self.acc + _dot(vt_v[self.hp, :, ks], self.p_prev[ks, :])
                self.kc += 1
                if self.kc == NC and self.p_prev is not None:
                    lsum = jnp.sum(l_v[self.l_prev], axis=0, keepdims=True)
                    o = self.acc * pl.reciprocal(lsum, approx=True)
                    store_o(self.hp, self.qbp, o)
                    ok = (lsum >= L_MIN) & (lsum <= L_MAX) & (jnp.abs(o) <= O_MAX)
                    bad_v[...] = jnp.maximum(bad_v[...], jnp.where(ok, 0.0, 1.0))
                if self.kc == NC and self.p_cur is not None:
                    l_v[1 - self.l_prev] = self.l

        class SlotPair:
            def __init__(self, t):
                self.t = t
                self.n = 0
                self.cur = None

            def chunk(self):
                if self.n >= 2 * NC:
                    return
                if self.n == 0:
                    self.cur = Slot(self.t, pa_v, pb_v, 1)
                elif self.n == NC:
                    self.cur = Slot(self.t + 1, pb_v, pa_v, 0)
                self.cur.chunk()
                self.n += 1

            def finish(self):
                while self.n < 2 * NC:
                    self.chunk()

        def run_slot(t, p_cur, p_prev, l_prev):
            sl = Slot(t, p_cur, p_prev, l_prev)
            for _ in range(NC):
                sl.chunk()

        st2 = st_v.reshape(3 * D * PITCH, EB)

        RU = 32
        NDC = D // RU

        def relayout_unit(w, i, dc):
            u = st2[pl.ds((w * D + dc * RU) * PITCH + i, RU, stride=PITCH), :]
            lo = pltpu.bitcast(u << 16, F32).astype(BF16)
            hi = pltpu.bitcast(u & jnp.uint32(0xFFFF0000), F32).astype(BF16)
            wB_v[w * HB + 2 * i, pl.ds(dc * RU, RU), :] = lo
            wB_v[w * HB + 2 * i + 1, pl.ds(dc * RU, RU), :] = hi

        ri = lax.broadcasted_iota(jnp.int32, (L, L), 0)
        ci = lax.broadcasted_iota(jnp.int32, (L, L), 1)
        mask = (ri < M) | (ri >= ci)

        def b_step(s, filler):
            r0 = pl.multiple_of(s * SEG, SEG)
            xs = x_v[pl.ds(r0, SEG), :].astype(F32)
            h = jnp.concatenate([mem_v[...], xs], axis=0)
            for hd in range(HB):
                q_s[hd] = _dot(h, wB_v[hd])
                k_s[hd] = _dot(h, wB_v[HB + hd]).astype(BF16)
                v_s[hd] = _dot(h, wB_v[2 * HB + hd]).astype(BF16)
                if hd % 2 == 1:
                    filler()
            pls = []
            for hd in range(HB):
                sc = _dot_nt(q_s[hd], k_s[hd]) * cB
                sc = jnp.where(mask, sc, -1e9)
                m = jnp.max(sc, axis=1, keepdims=True)
                p = jnp.exp2(sc - m)
                pls.append((p, jnp.sum(p, axis=1, keepdims=True)))
                if hd % 8 == 7:
                    filler()
            for hd in range(HB):
                p, l = pls[hd]
                o_s[hd] = _dot(p, v_s[hd]) * pl.reciprocal(l, approx=True)
                if hd % 8 == 7:
                    filler()
            out = jnp.zeros((L, D), F32)
            for hd in range(HB):
                out = out + _dot(o_s[hd], woB_v[hd * EB:(hd + 1) * EB, :])
                if hd % 4 == 3:
                    filler()
            b_v[pl.ds(r0, SEG), :] = out[M:, :]
            mem_v[...] = out[:M, :].astype(BF16).astype(F32)

        cp_mem.wait()
        mem_v[...] = mem0_v[...].astype(F32)

        with scope("P2_fast"):
            cp_gw.wait()
            once = jnp.minimum(jnp.maximum(jnp.max(pltpu.bitcast(gw_v[...].astype(F32), jnp.int32)), 1), 1)
            with scope("P2a_pre"):
                run_slot(0, pa_v, None, 1)
                run_slot(1, pb_v, pa_v, 0)
                with scope("P2a_wwait"):
                    for w in range(3):
                        cp_w[w].wait()
                for w in range(3):
                    def pre_body(_, c, w=w):
                        units = [(i, dc) for i in range(NP) for dc in range(NDC)]
                        sp = SlotPair(2 + 2 * w)
                        for n in range(2 * NC):
                            sp.chunk()
                            for i, dc in units[n * len(units) // (2 * NC):(n + 1) * len(units) // (2 * NC)]:
                                relayout_unit(w, i, dc)
                        return c

                    lax.fori_loop(0, once, pre_body, 0)
                cp_woB.wait()

            with scope("P2b_fused"):
                def fused_body(s, c):
                    sp = SlotPair(2 + 2 * NPRE + 2 * s)
                    b_step(s, sp.chunk)
                    sp.finish()
                    return c

                lax.fori_loop(0, NFUSE, fused_body, 0, unroll=UNROLL)
                run_slot(NBLK, None, pb_v, 1)


        @pl.when(jnp.max(bad_v[...]) != 0.0)
        def _true_max():
            def body(it, c):
                h, qb = it // NQ, it % NQ
                g, qtm = masked_q(h, qb)

                def max_body(kc, m):
                    ks = pl.ds(pl.multiple_of(kc * 256, 256), 256)
                    s = _dot(k_v[g, ks, :], qtm)
                    return jnp.maximum(m, jnp.max(s, axis=0, keepdims=True))

                m = lax.fori_loop(0, S // 256, max_body, jnp.full((1, BQ), -jnp.inf, F32))

                def pv_body(kc, carry):
                    l, acc = carry
                    ks = pl.ds(pl.multiple_of(kc * 256, 256), 256)
                    s = _dot(k_v[g, ks, :], qtm)
                    p = jnp.exp2(s - m)
                    l = l + jnp.sum(p, axis=0, keepdims=True)
                    acc = acc + _dot(vt_v[h, :, ks], p.astype(BF16))
                    return l, acc

                l, acc = lax.fori_loop(0, S // 256, pv_body,
                                       (jnp.zeros((1, BQ), F32), jnp.zeros((DA, BQ), F32)))
                store_o(h, qb, acc * (1.0 / l))
                return c

            lax.fori_loop(0, NBLK, body, 0)

        with scope("P3_last"):
            cp_wo.wait()
            gw = gw_v[...].astype(F32)

            def out_copy(j):
                r0 = pl.multiple_of(j * XC, XC)
                return pltpu.make_async_copy(o_v.at[pl.ds(r0, XC)], out_hbm.at[pl.ds(r0, XC)], osems.at[j])

            RB = 128
            b_v[S - SEG:S, :] = jnp.zeros((SEG, D), F32)

            def mix(gate, a, b):
                return (gate * a + (1.0 - gate) * b).astype(o_v.dtype)

            def last_body(j, c):
                done = []

                def filler():
                    i = len(done)
                    if i < XC // RB:
                        done.append(i)
                        r0 = pl.multiple_of(j * XC + i * RB, RB)
                        xs = x_v[pl.ds(r0, RB), :].astype(F32)
                        gate = jax.nn.sigmoid(jnp.sum(xs * gw, axis=1, keepdims=True))
                        a = _dot_tn(ot_v[:, pl.ds(r0, RB)], wo_v[...])
                        o_v[pl.ds(r0, RB), :] = mix(gate, a, b_v[pl.ds(r0, RB), :])
                        if i == XC // RB - 1:
                            alast_v[...] = a[RB - SEG:, :]
                            glast_v[...] = gate[RB - SEG:, :]

                b_step(NFUSE + j, filler)

                @pl.when(j < NXC - 1)
                def _():
                    out_copy(j).start()

                return c

            lax.fori_loop(0, NXC, last_body, 0)
            o_v[S - SEG:S, :] = mix(glast_v[...], alast_v[...], b_v[S - SEG:S, :])
            out_copy(NXC - 1).start()
            for j in range(NXC):
                out_copy(j).wait()

    return kernel


def _noscope(name):
    import contextlib
    return contextlib.nullcontext()


SCOPE = _noscope


@functools.partial(jax.jit, static_argnames=("B_seg_len",))
def pallas_gated_mix__mha_block__memory_aug_recurrent_mem_tr__prompt_kernel(
    A_x, A_wqkv, A_wo, B_x, B_mem0, B_Wq, B_Wk, B_Wv, B_Wo, B_seg_len, gate_w,
):
    del B_x
    Bsz, S, D = A_x.shape
    assert Bsz == 1
    HA = 32
    _, HB, EB = B_Wq.shape
    M = B_mem0.shape[1]
    SEG = int(B_seg_len)
    L = M + SEG

    x = A_x.reshape(S, D)
    kernel = _make_kernel(S, D, HA, HB, EB, M, SEG, SCOPE)
    any_spec = pl.BlockSpec(memory_space=pl.ANY)
    out = pl.pallas_call(
        kernel,
        out_shape=jax.ShapeDtypeStruct((S, D), A_x.dtype),
        in_specs=[any_spec] * 9,
        out_specs=any_spec,
        scratch_shapes=[
            pltpu.VMEM((M, D), B_mem0.dtype),
            pltpu.VMEM((1, D), gate_w.dtype),
            pltpu.VMEM((S, D), BF16),
            pltpu.VMEM((3, D, D), BF16),
            pltpu.VMEM((D, D), BF16),
            pltpu.VMEM((3, D, 24, EB), jnp.uint32),
            pltpu.VMEM((HB * EB, D), BF16),
            pltpu.VMEM((3 * HB, D, EB), BF16),
            pltpu.VMEM((D, D), BF16),
            pltpu.VMEM((D, D), BF16),
            pltpu.VMEM((D // 128, S, 128), BF16),
            pltpu.VMEM((D, S), BF16),
            pltpu.VMEM((HA, D // HA, S), BF16),
            pltpu.VMEM((S, 512), BF16),
            pltpu.VMEM((S, 512), BF16),
            pltpu.VMEM((D, S), BF16),
            pltpu.VMEM((S, D), F32),
            pltpu.VMEM((S, D), A_x.dtype),
            pltpu.VMEM((M, D), F32),
            pltpu.VMEM((2, 8, 512), F32),
            pltpu.VMEM((D // HA, 512), F32),
            pltpu.VMEM((SEG, D), F32),
            pltpu.VMEM((SEG, 1), F32),
            pltpu.VMEM((HB, L, EB), F32),
            pltpu.VMEM((HB, L, EB), BF16),
            pltpu.VMEM((HB, L, EB), BF16),
            pltpu.VMEM((HB, L, EB), F32),
            pltpu.SemaphoreType.DMA((10 + S // 512,)),
            pltpu.SemaphoreType.DMA((S // 512,)),
        ],
        compiler_params=pltpu.CompilerParams(vmem_limit_bytes=100 * 1024 * 1024),
    )(
        x, A_wqkv, A_wo, B_mem0.reshape(M, D),
        B_Wq, B_Wk, B_Wv,
        B_Wo.reshape(HB * EB, D), gate_w.reshape(1, D),
    )
    return out.reshape(Bsz, S, D)
```

```python
import functools
import math

import jax
import jax.numpy as jnp
from jax import lax
from jax.experimental import pallas as pl
from jax.experimental.pallas import tpu as pltpu

F32 = jnp.float32
BF16 = jnp.bfloat16
LOG2E = math.log2(math.e)

L_MIN = 2.0 ** -32
L_MAX = 2.0 ** 64
O_MAX = 3.0e38
UNROLL = 3
FILL = (18, 4, 4, 6)
FILL_LAST = (16, 4, 4, 8)


U32 = jnp.uint32


def _unpk(words):
    return pltpu.bitcast(words, BF16)


def _pk(vals):
    return pltpu.bitcast(vals, U32)


def _dot(a, b):
    return lax.dot_general(a, b, (((1,), (0,)), ((), ())), preferred_element_type=F32)


def _dot_nt(a, b):
    return lax.dot_general(a, b, (((1,), (1,)), ((), ())), preferred_element_type=F32)


def _dot_tn(a, b):
    return lax.dot_general(a, b, (((0,), (0,)), ((), ())), preferred_element_type=F32)


def _dot_tt(a, b):
    return lax.dot_general(a, b, (((0,), (1,)), ((), ())), preferred_element_type=F32)


def _make_kernel(S, D, HA, HB, EB, M, SEG):
    DA = D // HA
    HPG = 128 // DA
    NG = D // 128
    BQ = 512
    BK = 128
    NC = S // BK
    NQ = S // BQ
    NBLK = HA * NQ
    NSEG = S // SEG
    L = M + SEG
    NP = HB // 2
    XC = 512
    NXC = S // XC
    PITCH = 24
    NPRE = 3
    NFUSE = NSEG - NXC
    assert 2 + 2 * NPRE + 2 * NFUSE == NBLK
    cA = (DA ** -0.5) * LOG2E
    cB = (EB ** -0.5) * LOG2E

    def kernel(x_hbm, wqkv_hbm, wo_hbm, mem0_hbm, wq_hbm, wk_hbm, wv_hbm, woB_hbm, gw_hbm,
               out_hbm,
               mem0_v, gw1_v, gw_v, x_v, wqkv_v, wo_v, st_v, woB_v, wB_v,
               k_v, qt_v, vt_v, pa_v, pb_v, ot_v, b_v, o_v, mem_v, l_v, bad_v, alast_v, g_v,
               q_s, k_s, v_s, o_s, sems, osems):
        x_w, wqkv_w = x_hbm.bitcast(U32), wqkv_hbm.bitcast(U32)
        cp_wa = [pltpu.make_async_copy(wqkv_w.at[:, pl.ds(i * D, D)], wqkv_v.at[i], sems.at[i]) for i in range(3)]

        def x_copy(c):
            cs = pl.ds(pl.multiple_of(c * (XC // 2), XC // 2), XC // 2)
            return pltpu.make_async_copy(x_w.at[cs], x_v.at[cs], sems.at[3 + c])

        cp_x = [x_copy(c) for c in range(NXC)]
        cp_w = [
            pltpu.make_async_copy(w.bitcast(jnp.uint32), st_v.at[i, :, pl.ds(0, NP), :], sems.at[3 + NXC + i])
            for i, w in enumerate((wq_hbm, wk_hbm, wv_hbm))
        ]
        cp_woB = pltpu.make_async_copy(woB_hbm.bitcast(U32), woB_v, sems.at[6 + NXC])
        cp_wo = pltpu.make_async_copy(wo_hbm.bitcast(U32), wo_v, sems.at[7 + NXC])
        cp_mem = pltpu.make_async_copy(mem0_hbm, mem0_v, sems.at[8 + NXC])
        cp_gw = pltpu.make_async_copy(gw_hbm, gw1_v, sems.at[9 + NXC])
        for cp in [cp_wa[1]] + cp_x + [cp_wa[0], cp_wa[2], cp_mem, cp_gw]:
            cp.start()
        st_v[:, :, NP:PITCH, :] = jnp.zeros((3, D, PITCH - NP, EB), U32)
        for cp in cp_w + [cp_woB, cp_wo]:
            cp.start()

        cp_wa[1].wait()

        def k_body(c, carry):
            cw = pl.ds(pl.multiple_of(c * (XC // 2), XC // 2), XC // 2)
            x_copy(c).wait()
            xc = _unpk(x_v[cw, :])
            for g in range(NG):
                k_v[g, cw, :] = _pk(_dot(xc, _unpk(wqkv_v[1, :, g * 128:(g + 1) * 128])).astype(BF16))
            return carry

        lax.fori_loop(0, NXC, k_body, 0)
        cp_wa[0].wait()
        cp_wa[2].wait()

        def qv_body(c, carry):
            cs = pl.ds(pl.multiple_of(c * XC, XC), XC)
            cw = pl.ds(pl.multiple_of(c * (XC // 2), XC // 2), XC // 2)
            xc = _unpk(x_v[cw, :])
            qt_v[:, cs] = _pk((_dot_tt(_unpk(wqkv_v[0]), xc) * cA).astype(BF16))
            vc = _pk(_dot_tt(_unpk(wqkv_v[2]), xc).astype(BF16))
            for hh in range(HA):
                vt_v[hh, :, cs] = vc[hh * (DA // 2):(hh + 1) * (DA // 2), :]
            return carry

        lax.fori_loop(0, NXC, qv_body, 0)
        bad_v[...] = jnp.zeros_like(bad_v)

        def masked_q(h, qb):
            g = h // HPG
            j = h % HPG
            q0 = pl.multiple_of(qb * BQ, BQ)
            g0 = pl.multiple_of(g * 64, 64)
            qt = qt_v[pl.ds(g0, 64), pl.ds(q0, BQ)]
            row = lax.broadcasted_iota(jnp.int32, (64, BQ), 0)
            keep = (row >= j * (DA // 2)) & (row < (j + 1) * (DA // 2))
            return g, _unpk(jnp.where(keep, qt, jnp.zeros_like(qt)))

        def store_o(h, qb, o):
            ot_v[pl.ds(pl.multiple_of(h * (DA // 2), DA // 2), DA // 2),
                 pl.ds(pl.multiple_of(qb * BQ, BQ), BQ)] = _pk(o.astype(BF16))

        class Slot:
            def __init__(self, t, p_cur, p_prev, l_prev):
                self.p_cur, self.p_prev, self.l_prev = p_cur, p_prev, l_prev
                self.kc = 0
                if p_cur is not None:
                    self.g, self.qtm = masked_q(t // NQ, t % NQ)
                    self.l = jnp.zeros((8, BQ), F32)
                if p_prev is not None:
                    self.hp, self.qbp = (t - 1) // NQ, (t - 1) % NQ
                    self.acc = jnp.zeros((DA, BQ), F32)

            def chunk(self):
                ks = pl.ds(self.kc * BK, BK)
                kw = pl.ds(self.kc * (BK // 2), BK // 2)
                if self.p_cur is not None:
                    p = jnp.exp2(_dot(_unpk(k_v[self.g, kw, :]), self.qtm))
                    self.l = self.l + p.reshape(BK // 8, 8, BQ).sum(axis=0)
                    self.p_cur[kw, :] = _pk(p.astype(BF16))
                if self.p_prev is not None:
                    self.acc = self.acc + _dot(_unpk(vt_v[self.hp, :, ks]), _unpk(self.p_prev[kw, :]))
                self.kc += 1
                if self.kc == NC and self.p_prev is not None:
                    lsum = jnp.sum(l_v[self.l_prev], axis=0, keepdims=True)
                    o = self.acc * pl.reciprocal(lsum, approx=True)
                    store_o(self.hp, self.qbp, o)
                    ok = (lsum >= L_MIN) & (lsum <= L_MAX) & (jnp.abs(o) <= O_MAX)
                    bad_v[...] = jnp.maximum(bad_v[...], jnp.where(ok, 0.0, 1.0))
                if self.kc == NC and self.p_cur is not None:
                    l_v[1 - self.l_prev] = self.l

        class SlotPair:
            def __init__(self, t):
                self.t = t
                self.n = 0
                self.cur = None

            def chunk(self):
                if self.n >= 2 * NC:
                    return
                if self.n == 0:
                    self.cur = Slot(self.t, pa_v, pb_v, 1)
                elif self.n == NC:
                    self.cur = Slot(self.t + 1, pb_v, pa_v, 0)
                self.cur.chunk()
                self.n += 1

            def finish(self):
                while self.n < 2 * NC:
                    self.chunk()

        def run_slot(t, p_cur, p_prev, l_prev):
            sl = Slot(t, p_cur, p_prev, l_prev)
            for _ in range(NC):
                sl.chunk()

        st2 = st_v.reshape(3 * D * PITCH, EB)

        RU = 32
        NDC = D // RU

        def relayout_unit(w, i, dc):
            u = st2[pl.ds((w * D + dc * RU) * PITCH + i, RU, stride=PITCH), :]
            lo = pltpu.bitcast(u << 16, F32).astype(BF16)
            hi = pltpu.bitcast(u & jnp.uint32(0xFFFF0000), F32).astype(BF16)
            wB_v[w * HB + 2 * i, pl.ds(dc * (RU // 2), RU // 2), :] = _pk(lo)
            wB_v[w * HB + 2 * i + 1, pl.ds(dc * (RU // 2), RU // 2), :] = _pk(hi)

        ri = lax.broadcasted_iota(jnp.int32, (L, L), 0)
        ci = lax.broadcasted_iota(jnp.int32, (L, L), 1)
        mask = (ri < M) | (ri >= ci)

        def gates(r0, xs):
            gate = jax.nn.sigmoid(jnp.sum(xs * gw_v[...], axis=1, keepdims=True))
            g_v[pl.ds(r0, xs.shape[0]), :] = jnp.broadcast_to(gate, (xs.shape[0], 128))

        def b_step(s, filler, fill, with_gates):
            def spread(stage, hd):
                return ((hd + 1) * fill[stage]) // HB - (hd * fill[stage]) // HB

            r0 = pl.multiple_of(s * SEG, SEG)
            xs = _unpk(x_v[pl.ds(pl.multiple_of(s * (SEG // 2), SEG // 2), SEG // 2), :]).astype(F32)
            if with_gates:
                gates(r0, xs)
            h = jnp.concatenate([mem_v[...], xs], axis=0)
            for hd in range(HB):
                q_s[hd] = _dot(h, _unpk(wB_v[hd]))
                k_s[hd] = _dot(h, _unpk(wB_v[HB + hd])).astype(BF16)
                v_s[hd] = _dot(h, _unpk(wB_v[2 * HB + hd])).astype(BF16)
                for _ in range(spread(0, hd)):
                    filler()
            pls = []
            for hd in range(HB):
                sc = _dot_nt(q_s[hd], k_s[hd]) * cB
                sc = jnp.where(mask, sc, -1e9)
                m = jnp.max(sc, axis=1, keepdims=True)
                p = jnp.exp2(sc - m)
                pls.append((p, jnp.sum(p, axis=1, keepdims=True)))
                for _ in range(spread(1, hd)):
                    filler()
            for hd in range(HB):
                p, l = pls[hd]
                o_s[hd] = _dot(p, v_s[hd]) * pl.reciprocal(l, approx=True)
                for _ in range(spread(2, hd)):
                    filler()
            out = jnp.zeros((L, D), F32)
            for hd in range(HB):
                out = out + _dot(o_s[hd], _unpk(woB_v[hd * (EB // 2):(hd + 1) * (EB // 2), :]))
                for _ in range(spread(3, hd)):
                    filler()
            b_v[pl.ds(r0, SEG), :] = out[M:, :]
            mem_v[...] = out[:M, :].astype(BF16).astype(F32)

        cp_mem.wait()
        mem_v[...] = mem0_v[...].astype(F32)

        cp_gw.wait()
        gw_v[...] = gw1_v[...].astype(F32).reshape(1, D)
        once = jnp.minimum(jnp.maximum(jnp.max(pltpu.bitcast(gw_v[...], jnp.int32)), 1), 1)
        run_slot(0, pa_v, None, 1)
        run_slot(1, pb_v, pa_v, 0)
        for w in range(3):
            cp_w[w].wait()
        for w in range(3):
            def pre_body(_, c, w=w):
                units = [(i, dc) for i in range(NP) for dc in range(NDC)]
                sp = SlotPair(2 + 2 * w)
                for n in range(2 * NC):
                    sp.chunk()
                    for i, dc in units[n * len(units) // (2 * NC):(n + 1) * len(units) // (2 * NC)]:
                        relayout_unit(w, i, dc)
                return c

            lax.fori_loop(0, once, pre_body, 0)
        cp_woB.wait()

        def fused_body(s, c):
            sp = SlotPair(2 + 2 * NPRE + 2 * s)
            b_step(s, sp.chunk, FILL, True)
            sp.finish()
            return c

        lax.fori_loop(0, NFUSE, fused_body, 0, unroll=UNROLL)
        gates(NFUSE * SEG, _unpk(x_v[NFUSE * SEG // 2:S // 2, :]).astype(F32))
        run_slot(NBLK, None, pb_v, 1)


        @pl.when(jnp.max(bad_v[...]) != 0.0)
        def _true_max():
            def body(it, c):
                h, qb = it // NQ, it % NQ
                g, qtm = masked_q(h, qb)

                def max_body(kc, m):
                    s = _dot(_unpk(k_v[g, pl.ds(pl.multiple_of(kc * 128, 128), 128), :]), qtm)
                    return jnp.maximum(m, jnp.max(s, axis=0, keepdims=True))

                m = lax.fori_loop(0, S // 256, max_body, jnp.full((1, BQ), -jnp.inf, F32))

                def pv_body(kc, carry):
                    l, acc = carry
                    ks = pl.ds(pl.multiple_of(kc * 256, 256), 256)
                    s = _dot(_unpk(k_v[g, pl.ds(pl.multiple_of(kc * 128, 128), 128), :]), qtm)
                    p = jnp.exp2(s - m)
                    l = l + jnp.sum(p, axis=0, keepdims=True)
                    acc = acc + _dot(_unpk(vt_v[h, :, ks]), p.astype(BF16))
                    return l, acc

                l, acc = lax.fori_loop(0, S // 256, pv_body,
                                       (jnp.zeros((1, BQ), F32), jnp.zeros((DA, BQ), F32)))
                store_o(h, qb, acc * (1.0 / l))
                return c

            lax.fori_loop(0, NBLK, body, 0)

        cp_wo.wait()

        def out_copy(j, tail):
            r0 = pl.multiple_of(j * XC + (XC - SEG) * tail, SEG)
            rows = pl.ds(r0, SEG if tail else XC - SEG)
            return pltpu.make_async_copy(o_v.at[rows], out_hbm.at[rows], osems.at[2 * j + tail])

        RB = 128
        PIECE_AT = (16, 19, 22, 25)
        b_v[S - SEG:S, :] = jnp.zeros((SEG, D), F32)

        def mix(gate, a, b):
            gate = jnp.concatenate([gate] * (D // 128), axis=1)
            return (gate * a + (1.0 - gate) * b).astype(o_v.dtype)

        def last_body(j, c):
            done = []

            calls = []

            def filler():
                calls.append(0)
                i = len(done)
                if len(calls) in PIECE_AT:
                    done.append(i)
                    r0 = pl.multiple_of(j * XC + i * RB, RB)
                    gate = g_v[pl.ds(r0, RB), :]
                    a = _dot_tn(_unpk(ot_v[:, pl.ds(r0, RB)]), _unpk(wo_v[...]))
                    o_v[pl.ds(r0, RB), :] = mix(gate, a, b_v[pl.ds(r0, RB), :])
                    if i == XC // RB - 1:
                        alast_v[...] = a[RB - SEG:, :]
                        out_copy(j, 0).start()

            b_step(NFUSE + j, filler, FILL_LAST, False)

            @pl.when(j < NXC - 1)
            def _():
                out_copy(j, 1).start()

            return c

        lax.fori_loop(0, NXC, last_body, 0)
        o_v[S - SEG:S, :] = mix(g_v[S - SEG:S, :], alast_v[...], b_v[S - SEG:S, :])
        out_copy(NXC - 1, 1).start()
        for j in range(NXC):
            out_copy(j, 0).wait()
            out_copy(j, 1).wait()

    return kernel


@functools.partial(jax.jit, static_argnames=("B_seg_len",))
def pallas_gated_mix__mha_block__memory_aug_recurrent_mem_tr__prompt_kernel(
    A_x, A_wqkv, A_wo, B_x, B_mem0, B_Wq, B_Wk, B_Wv, B_Wo, B_seg_len, gate_w,
):
    del B_x
    Bsz, S, D = A_x.shape
    assert Bsz == 1
    HA = 32
    _, HB, EB = B_Wq.shape
    M = B_mem0.shape[1]
    SEG = int(B_seg_len)
    L = M + SEG

    x = A_x.reshape(S, D)
    kernel = _make_kernel(S, D, HA, HB, EB, M, SEG)
    any_spec = pl.BlockSpec(memory_space=pl.ANY)
    out = pl.pallas_call(
        kernel,
        out_shape=jax.ShapeDtypeStruct((S, D), A_x.dtype),
        in_specs=[any_spec] * 9,
        out_specs=any_spec,
        scratch_shapes=[
            pltpu.VMEM((M, D), B_mem0.dtype),
            pltpu.VMEM((D,), gate_w.dtype),
            pltpu.VMEM((1, D), F32),
            pltpu.VMEM((S // 2, D), U32),
            pltpu.VMEM((3, D // 2, D), U32),
            pltpu.VMEM((D // 2, D), U32),
            pltpu.VMEM((3, D, 24, EB), jnp.uint32),
            pltpu.VMEM((HB * EB // 2, D), U32),
            pltpu.VMEM((3 * HB, D // 2, EB), U32),
            pltpu.VMEM((D // 128, S // 2, 128), U32),
            pltpu.VMEM((D // 2, S), U32),
            pltpu.VMEM((HA, D // HA // 2, S), U32),
            pltpu.VMEM((S // 2, 512), U32),
            pltpu.VMEM((S // 2, 512), U32),
            pltpu.VMEM((D // 2, S), U32),
            pltpu.VMEM((S, D), F32),
            pltpu.VMEM((S, D), A_x.dtype),
            pltpu.VMEM((M, D), F32),
            pltpu.VMEM((2, 8, 512), F32),
            pltpu.VMEM((D // HA, 512), F32),
            pltpu.VMEM((SEG, D), F32),
            pltpu.VMEM((S, 128), F32),
            pltpu.VMEM((HB, L, EB), F32),
            pltpu.VMEM((HB, L, EB), BF16),
            pltpu.VMEM((HB, L, EB), BF16),
            pltpu.VMEM((HB, L, EB), F32),
            pltpu.SemaphoreType.DMA((10 + S // 512,)),
            pltpu.SemaphoreType.DMA((2 * S // 512,)),
        ],
        compiler_params=pltpu.CompilerParams(vmem_limit_bytes=100 * 1024 * 1024),
    )(
        x, A_wqkv, A_wo, B_mem0.reshape(M, D),
        B_Wq, B_Wk, B_Wv,
        B_Wo.reshape(HB * EB, D), gate_w,
    )
    return out.reshape(Bsz, S, D)
```

```python
import functools
import math

import jax
import jax.numpy as jnp
from jax import lax
from jax.experimental import pallas as pl
from jax.experimental.pallas import tpu as pltpu

F32 = jnp.float32
BF16 = jnp.bfloat16
U32 = jnp.uint32
LOG2E = math.log2(math.e)

L_MIN = 1.0
L_MAX = 2.0 ** 64
O_MAX = 3.0e38

BQ = 512
BK = 128
XC = 512
PITCH = 24
UNROLL = 3
FILL = (18, 4, 4, 6)
FILL_LAST = (16, 4, 4, 8)
PIECE_AT = (16, 19, 22, 25)


def _unpk(words):
    return pltpu.bitcast(words, BF16)


def _pk(vals):
    return pltpu.bitcast(vals, U32)


def _dot(a, b):
    return lax.dot_general(a, b, (((1,), (0,)), ((), ())), preferred_element_type=F32)


def _dot_nt(a, b):
    return lax.dot_general(a, b, (((1,), (1,)), ((), ())), preferred_element_type=F32)


def _dot_tn(a, b):
    return lax.dot_general(a, b, (((0,), (0,)), ((), ())), preferred_element_type=F32)


def _dot_tt(a, b):
    return lax.dot_general(a, b, (((0,), (1,)), ((), ())), preferred_element_type=F32)


def _make_kernel(S, D, HA, HB, EB, M, SEG):
    DA = D // HA
    HPG = 128 // DA
    NG = D // 128
    NC = S // BK
    NQ = S // BQ
    NBLK = HA * NQ
    NSEG = S // SEG
    L = M + SEG
    NP = HB // 2
    NXC = S // XC
    NPRE = 3
    NFUSE = NSEG - NXC
    assert 2 + 2 * NPRE + 2 * NFUSE == NBLK and NFUSE % UNROLL == 0
    assert DA == 16 and EB == 128 and NP <= PITCH and sum(FILL) == sum(FILL_LAST) == 2 * NC
    cA = (DA ** -0.5) * LOG2E
    cB = (EB ** -0.5) * LOG2E

    def kernel(x_hbm, wqkv_hbm, wo_hbm, mem0_hbm, wq_hbm, wk_hbm, wv_hbm, woB_hbm, gw_hbm,
               out_hbm,
               mem0_v, gw1_v, gw_v, x_v, wqkv_v, wo_v, st_v, woB_v, wB_v,
               k_v, qt_v, vt_v, pa_v, pb_v, ot_v, b_v, o_v, mem_v, l_v, bad_v, alast_v, g_v,
               q_s, k_s, v_s, o_s, sems, osems):
        x_w, wqkv_w = x_hbm.bitcast(U32), wqkv_hbm.bitcast(U32)
        cp_wa = [pltpu.make_async_copy(wqkv_w.at[:, pl.ds(i * D, D)], wqkv_v.at[i], sems.at[i]) for i in range(3)]

        def x_copy(c):
            cs = pl.ds(pl.multiple_of(c * (XC // 2), XC // 2), XC // 2)
            return pltpu.make_async_copy(x_w.at[cs], x_v.at[cs], sems.at[3 + c])

        cp_x = [x_copy(c) for c in range(NXC)]
        cp_w = [
            pltpu.make_async_copy(w.bitcast(U32), st_v.at[i, :, pl.ds(0, NP), :], sems.at[3 + NXC + i])
            for i, w in enumerate((wq_hbm, wk_hbm, wv_hbm))
        ]
        cp_woB = pltpu.make_async_copy(woB_hbm.bitcast(U32), woB_v, sems.at[6 + NXC])
        cp_wo = pltpu.make_async_copy(wo_hbm.bitcast(U32), wo_v, sems.at[7 + NXC])
        cp_mem = pltpu.make_async_copy(mem0_hbm, mem0_v, sems.at[8 + NXC])
        cp_gw = pltpu.make_async_copy(gw_hbm, gw1_v, sems.at[9 + NXC])
        for cp in [cp_wa[1]] + cp_x + [cp_wa[0], cp_wa[2], cp_mem, cp_gw]:
            cp.start()
        st_v[:, :, NP:PITCH, :] = jnp.zeros((3, D, PITCH - NP, EB), U32)
        for cp in cp_w + [cp_woB, cp_wo]:
            cp.start()

        cp_wa[1].wait()

        def k_body(c, carry):
            cw = pl.ds(pl.multiple_of(c * (XC // 2), XC // 2), XC // 2)
            x_copy(c).wait()
            xc = _unpk(x_v[cw, :])
            for g in range(NG):
                k_v[g, cw, :] = _pk(_dot(xc, _unpk(wqkv_v[1, :, g * 128:(g + 1) * 128])).astype(BF16))
            return carry

        lax.fori_loop(0, NXC, k_body, 0)
        cp_wa[0].wait()
        cp_wa[2].wait()

        def qv_body(c, carry):
            cs = pl.ds(pl.multiple_of(c * XC, XC), XC)
            cw = pl.ds(pl.multiple_of(c * (XC // 2), XC // 2), XC // 2)
            xc = _unpk(x_v[cw, :])
            qt_v[:, cs] = _pk((_dot_tt(_unpk(wqkv_v[0]), xc) * cA).astype(BF16))
            vc = _pk(_dot_tt(_unpk(wqkv_v[2]), xc).astype(BF16))
            for hh in range(HA):
                vt_v[hh, :, cs] = vc[hh * (DA // 2):(hh + 1) * (DA // 2), :]
            return carry

        lax.fori_loop(0, NXC, qv_body, 0)
        bad_v[...] = jnp.zeros_like(bad_v)

        def masked_q(h, qb):
            g = h // HPG
            j = h % HPG
            q0 = pl.multiple_of(qb * BQ, BQ)
            g0 = pl.multiple_of(g * 64, 64)
            qt = qt_v[pl.ds(g0, 64), pl.ds(q0, BQ)]
            row = lax.broadcasted_iota(jnp.int32, (64, BQ), 0)
            keep = (row >= j * (DA // 2)) & (row < (j + 1) * (DA // 2))
            return g, _unpk(jnp.where(keep, qt, jnp.zeros_like(qt)))

        def store_o(h, qb, o):
            ot_v[pl.ds(pl.multiple_of(h * (DA // 2), DA // 2), DA // 2),
                 pl.ds(pl.multiple_of(qb * BQ, BQ), BQ)] = _pk(o.astype(BF16))

        class Slot:
            def __init__(self, t, p_cur, p_prev, l_prev):
                self.p_cur, self.p_prev, self.l_prev = p_cur, p_prev, l_prev
                self.kc = 0
                if p_cur is not None:
                    self.g, self.qtm = masked_q(t // NQ, t % NQ)
                    self.l = jnp.zeros((8, BQ), F32)
                if p_prev is not None:
                    self.hp, self.qbp = (t - 1) // NQ, (t - 1) % NQ
                    self.acc = jnp.zeros((DA, BQ), F32)

            def chunk(self):
                ks = pl.ds(self.kc * BK, BK)
                kw = pl.ds(self.kc * (BK // 2), BK // 2)
                if self.p_cur is not None:
                    p = jnp.exp2(_dot(_unpk(k_v[self.g, kw, :]), self.qtm))
                    self.l = self.l + p.reshape(BK // 8, 8, BQ).sum(axis=0)
                    self.p_cur[kw, :] = _pk(p.astype(BF16))
                if self.p_prev is not None:
                    self.acc = self.acc + _dot(_unpk(vt_v[self.hp, :, ks]), _unpk(self.p_prev[kw, :]))
                self.kc += 1
                if self.kc == NC and self.p_prev is not None:
                    lsum = jnp.sum(l_v[self.l_prev], axis=0, keepdims=True)
                    o = self.acc * pl.reciprocal(lsum, approx=True)
                    store_o(self.hp, self.qbp, o)
                    ok = (lsum >= L_MIN) & (lsum <= L_MAX) & (jnp.abs(o) <= O_MAX)
                    bad_v[...] = jnp.maximum(bad_v[...], jnp.where(ok, 0.0, 1.0))
                if self.kc == NC and self.p_cur is not None:
                    l_v[1 - self.l_prev] = self.l

        class SlotPair:
            def __init__(self, t):
                self.t = t
                self.n = 0
                self.cur = None

            def chunk(self):
                if self.n >= 2 * NC:
                    return
                if self.n == 0:
                    self.cur = Slot(self.t, pa_v, pb_v, 1)
                elif self.n == NC:
                    self.cur = Slot(self.t + 1, pb_v, pa_v, 0)
                self.cur.chunk()
                self.n += 1

            def finish(self):
                while self.n < 2 * NC:
                    self.chunk()

        def run_slot(t, p_cur, p_prev, l_prev):
            sl = Slot(t, p_cur, p_prev, l_prev)
            for _ in range(NC):
                sl.chunk()

        st2 = st_v.reshape(3 * D * PITCH, EB)
        RU = 32
        NDC = D // RU

        def relayout_unit(w, i, dc):
            u = st2[pl.ds((w * D + dc * RU) * PITCH + i, RU, stride=PITCH), :]
            lo = pltpu.bitcast(u << 16, F32).astype(BF16)
            hi = pltpu.bitcast(u & U32(0xFFFF0000), F32).astype(BF16)
            wB_v[w * HB + 2 * i, pl.ds(dc * (RU // 2), RU // 2), :] = _pk(lo)
            wB_v[w * HB + 2 * i + 1, pl.ds(dc * (RU // 2), RU // 2), :] = _pk(hi)

        ri = lax.broadcasted_iota(jnp.int32, (L, L), 0)
        ci = lax.broadcasted_iota(jnp.int32, (L, L), 1)
        mask = (ri < M) | (ri >= ci)

        def gates(r0, xs):
            gate = jax.nn.sigmoid(jnp.sum(xs * gw_v[...], axis=1, keepdims=True))
            g_v[pl.ds(r0, xs.shape[0]), :] = jnp.broadcast_to(gate, (xs.shape[0], 128))

        def b_step(s, filler, fill, with_gates):
            def spread(stage, hd):
                return ((hd + 1) * fill[stage]) // HB - (hd * fill[stage]) // HB

            r0 = pl.multiple_of(s * SEG, SEG)
            xs = _unpk(x_v[pl.ds(pl.multiple_of(s * (SEG // 2), SEG // 2), SEG // 2), :]).astype(F32)
            if with_gates:
                gates(r0, xs)
            h = jnp.concatenate([mem_v[...], xs], axis=0)
            for hd in range(HB):
                q_s[hd] = _dot(h, _unpk(wB_v[hd]))
                k_s[hd] = _dot(h, _unpk(wB_v[HB + hd])).astype(BF16)
                v_s[hd] = _dot(h, _unpk(wB_v[2 * HB + hd])).astype(BF16)
                for _ in range(spread(0, hd)):
                    filler()
            pls = []
            for hd in range(HB):
                sc = _dot_nt(q_s[hd], k_s[hd]) * cB
                sc = jnp.where(mask, sc, -1e9 * LOG2E)
                m = jnp.max(sc, axis=1, keepdims=True)
                p = jnp.exp2(sc - m)
                pls.append((p, jnp.sum(p, axis=1, keepdims=True)))
                for _ in range(spread(1, hd)):
                    filler()
            for hd in range(HB):
                p, l = pls[hd]
                o_s[hd] = _dot(p, v_s[hd]) * pl.reciprocal(l, approx=True)
                for _ in range(spread(2, hd)):
                    filler()
            out = jnp.zeros((L, D), F32)
            for hd in range(HB):
                out = out + _dot(o_s[hd], _unpk(woB_v[hd * (EB // 2):(hd + 1) * (EB // 2), :]))
                for _ in range(spread(3, hd)):
                    filler()
            b_v[pl.ds(r0, SEG), :] = out[M:, :]
            mem_v[...] = out[:M, :].astype(BF16).astype(F32)

        cp_mem.wait()
        mem_v[...] = mem0_v[...].astype(F32)

        cp_gw.wait()
        gw_v[...] = gw1_v[...].astype(F32).reshape(1, D)
        once = jnp.minimum(jnp.maximum(jnp.max(pltpu.bitcast(gw_v[...], jnp.int32)), 1), 1)
        run_slot(0, pa_v, None, 1)
        run_slot(1, pb_v, pa_v, 0)
        for w in range(3):
            cp_w[w].wait()
        for w in range(3):
            def pre_body(_, c, w=w):
                units = [(i, dc) for i in range(NP) for dc in range(NDC)]
                sp = SlotPair(2 + 2 * w)
                for n in range(2 * NC):
                    sp.chunk()
                    for i, dc in units[n * len(units) // (2 * NC):(n + 1) * len(units) // (2 * NC)]:
                        relayout_unit(w, i, dc)
                return c

            lax.fori_loop(0, once, pre_body, 0)
        cp_woB.wait()

        def fused_body(s, c):
            sp = SlotPair(2 + 2 * NPRE + 2 * s)
            b_step(s, sp.chunk, FILL, True)
            sp.finish()
            return c

        lax.fori_loop(0, NFUSE, fused_body, 0, unroll=UNROLL)
        gates(NFUSE * SEG, _unpk(x_v[NFUSE * SEG // 2:S // 2, :]).astype(F32))
        run_slot(NBLK, None, pb_v, 1)

        @pl.when(jnp.max(bad_v[...]) != 0.0)
        def _true_max():
            def body(it, c):
                h, qb = it // NQ, it % NQ
                g, qtm = masked_q(h, qb)

                def max_body(kc, m):
                    s = _dot(_unpk(k_v[g, pl.ds(pl.multiple_of(kc * 128, 128), 128), :]), qtm)
                    return jnp.maximum(m, jnp.max(s, axis=0, keepdims=True))

                m = lax.fori_loop(0, S // 256, max_body, jnp.full((1, BQ), -jnp.inf, F32))

                def pv_body(kc, carry):
                    l, acc = carry
                    ks = pl.ds(pl.multiple_of(kc * 256, 256), 256)
                    s = _dot(_unpk(k_v[g, pl.ds(pl.multiple_of(kc * 128, 128), 128), :]), qtm)
                    p = jnp.exp2(s - m)
                    l = l + jnp.sum(p, axis=0, keepdims=True)
                    acc = acc + _dot(_unpk(vt_v[h, :, ks]), p.astype(BF16))
                    return l, acc

                l, acc = lax.fori_loop(0, S // 256, pv_body,
                                       (jnp.zeros((1, BQ), F32), jnp.zeros((DA, BQ), F32)))
                store_o(h, qb, acc * (1.0 / l))
                return c

            lax.fori_loop(0, NBLK, body, 0)

        cp_wo.wait()

        def out_copy(j, tail):
            r0 = pl.multiple_of(j * XC + (XC - SEG) * tail, SEG)
            rows = pl.ds(r0, SEG if tail else XC - SEG)
            return pltpu.make_async_copy(o_v.at[rows], out_hbm.at[rows], osems.at[2 * j + tail])

        RB = 128
        b_v[S - SEG:S, :] = jnp.zeros((SEG, D), F32)

        def mix(gate, a, b):
            gate = jnp.concatenate([gate] * (D // 128), axis=1)
            return (gate * a + (1.0 - gate) * b).astype(o_v.dtype)

        def last_body(j, c):
            done, calls = [], []

            def filler():
                calls.append(0)
                i = len(done)
                if len(calls) in PIECE_AT:
                    done.append(i)
                    r0 = pl.multiple_of(j * XC + i * RB, RB)
                    gate = g_v[pl.ds(r0, RB), :]
                    a = _dot_tn(_unpk(ot_v[:, pl.ds(r0, RB)]), _unpk(wo_v[...]))
                    o_v[pl.ds(r0, RB), :] = mix(gate, a, b_v[pl.ds(r0, RB), :])
                    if i == XC // RB - 1:
                        alast_v[...] = a[RB - SEG:, :]
                        out_copy(j, 0).start()

            b_step(NFUSE + j, filler, FILL_LAST, False)

            @pl.when(j < NXC - 1)
            def _():
                out_copy(j, 1).start()

            return c

        lax.fori_loop(0, NXC, last_body, 0)
        o_v[S - SEG:S, :] = mix(g_v[S - SEG:S, :], alast_v[...], b_v[S - SEG:S, :])
        out_copy(NXC - 1, 1).start()
        for j in range(NXC):
            out_copy(j, 0).wait()
            out_copy(j, 1).wait()

    return kernel


@functools.partial(jax.jit, static_argnames=("B_seg_len",))
def pallas_gated_mix__mha_block__memory_aug_recurrent_mem_tr__prompt_kernel(
    A_x, A_wqkv, A_wo, B_x, B_mem0, B_Wq, B_Wk, B_Wv, B_Wo, B_seg_len, gate_w,
):
    del B_x
    Bsz, S, D = A_x.shape
    assert Bsz == 1
    assert all(a.dtype == BF16 for a in (A_x, A_wqkv, A_wo, B_Wq, B_Wk, B_Wv, B_Wo))
    HA = 32
    _, HB, EB = B_Wq.shape
    M = B_mem0.shape[1]
    SEG = int(B_seg_len)
    L = M + SEG

    x = A_x.reshape(S, D)
    kernel = _make_kernel(S, D, HA, HB, EB, M, SEG)
    any_spec = pl.BlockSpec(memory_space=pl.ANY)
    out = pl.pallas_call(
        kernel,
        out_shape=jax.ShapeDtypeStruct((S, D), A_x.dtype),
        in_specs=[any_spec] * 9,
        out_specs=any_spec,
        scratch_shapes=[
            pltpu.VMEM((M, D), B_mem0.dtype),
            pltpu.VMEM((D,), gate_w.dtype),
            pltpu.VMEM((1, D), F32),
            pltpu.VMEM((S // 2, D), U32),
            pltpu.VMEM((3, D // 2, D), U32),
            pltpu.VMEM((D // 2, D), U32),
            pltpu.VMEM((3, D, PITCH, EB), U32),
            pltpu.VMEM((HB * EB // 2, D), U32),
            pltpu.VMEM((3 * HB, D // 2, EB), U32),
            pltpu.VMEM((D // 128, S // 2, 128), U32),
            pltpu.VMEM((D // 2, S), U32),
            pltpu.VMEM((HA, D // HA // 2, S), U32),
            pltpu.VMEM((S // 2, BQ), U32),
            pltpu.VMEM((S // 2, BQ), U32),
            pltpu.VMEM((D // 2, S), U32),
            pltpu.VMEM((S, D), F32),
            pltpu.VMEM((S, D), A_x.dtype),
            pltpu.VMEM((M, D), F32),
            pltpu.VMEM((2, 8, BQ), F32),
            pltpu.VMEM((D // HA, BQ), F32),
            pltpu.VMEM((SEG, D), F32),
            pltpu.VMEM((S, 128), F32),
            pltpu.VMEM((HB, L, EB), F32),
            pltpu.VMEM((HB, L, EB), BF16),
            pltpu.VMEM((HB, L, EB), BF16),
            pltpu.VMEM((HB, L, EB), F32),
            pltpu.SemaphoreType.DMA((10 + S // XC,)),
            pltpu.SemaphoreType.DMA((2 * S // XC,)),
        ],
        compiler_params=pltpu.CompilerParams(vmem_limit_bytes=100 * 1024 * 1024),
    )(
        x, A_wqkv, A_wo, B_mem0.reshape(M, D),
        B_Wq, B_Wk, B_Wv,
        B_Wo.reshape(HB * EB, D), gate_w,
    )
    return out.reshape(Bsz, S, D)
```
